```python
import os as _os
_os.environ.setdefault("JAX_PLATFORMS", "cpu")
import jax
import jax.numpy as jnp

def _softmax(x, axis=-1):
    return jax.nn.softmax(x, axis=axis)
def _gelu(x):
    return jax.nn.gelu(x, approximate=True)
def _silu(x):
    return jax.nn.silu(x)
def _sigmoid(x):
    return jax.nn.sigmoid(x)
def _layernorm(x, axis=-1, eps=1e-5):
    m = jnp.mean(x, axis=axis, keepdims=True)
    v = jnp.var(x, axis=axis, keepdims=True)
    return (x - m) / jnp.sqrt(v + eps)
def _scatter_add(tgt, idx, src, axis=0):
    return tgt.at[idx].add(src)
def _segment_sum(src, seg, n):
    return jax.ops.segment_sum(src, seg, n)
class _Rng:
    def __init__(self, key):
        self._k = key
    def _next(self):
        self._k, sub = jax.random.split(self._k)
        return sub
    def normal(self, shape):
        return jax.random.normal(self._next(), shape, dtype=jnp.bfloat16)
    def randint(self, lo, hi, shape):
        return jax.random.randint(self._next(), shape, lo, hi, dtype=jnp.int32)
    def uniform(self, shape, lo=0.0, hi=1.0):
        return jax.random.uniform(self._next(), shape, jnp.bfloat16, lo, hi)
    def permutation(self, n):
        return jax.random.permutation(self._next(), n)


kernel_name = 'sequential_preLN__mha_block__moe_arch_mod__prompt'

def setup_inputs():
    _rng = _Rng(jax.random.key(int.from_bytes(__import__("os").urandom(4), "little")))
    _w = (lambda a: (lambda t: t.astype(jnp.bfloat16) if jnp.issubdtype(t.dtype, jnp.floating) else t)(jnp.asarray(a)))
    def _A_setup():
        B, S, D, H = 1, 2048, 640, 32
        return {
            "x": _w((lambda *s: _rng.normal(s) * 0.05)(B, S, D)),
            "wqkv": _w((lambda *s: _rng.normal(s) * 0.05)(D, 3 * D)),
            "wo": _w((lambda *s: _rng.normal(s) * 0.05)(D, D)),
        }
    _A_in = _A_setup()

    def _B_setup():
        B, S, D, F, C = 1, 2048, 640, 1536, 1
        return {
            "x": _w((lambda *s: _rng.normal(s) * 0.05)(B, S, D)),
            "w_r": _w((lambda *s: _rng.normal(s) * 0.05)(D)),
            "w_gate": _w((lambda *s: _rng.normal(s) * 0.05)(D, F)),
            "w_up": _w((lambda *s: _rng.normal(s) * 0.05)(D, F)),
            "w_down": _w((lambda *s: _rng.normal(s) * 0.05)(F, D)),
        }
    _B_in = _B_setup()

    return {
        "A_x": _A_in["x"],
        "A_wqkv": _A_in["wqkv"],
        "A_wo": _A_in["wo"],
        "B_x": _B_in["x"],
        "B_w_r": _B_in["w_r"],
        "B_w_gate": _B_in["w_gate"],
        "B_w_up": _B_in["w_up"],
        "B_w_down": _B_in["w_down"],
    }

def reference(A_x, A_wqkv, A_wo, B_x, B_w_r, B_w_gate, B_w_up, B_w_down):
    def _A_ref(x, wqkv, wo):
        B, S, D = x.shape
        H = 32
        Dh = D // H
        qkv = (lambda x, *d: x.transpose(*d))((x @ wqkv).reshape(B, S, 3, H, Dh), 2, 0, 3, 1, 4)
        q, k, v = qkv[0], qkv[1], qkv[2]
        scores = jnp.einsum("bhqd,bhkd->bhqk", q, k) * (Dh ** -0.5)
        p = _softmax(scores, axis=-1)
        o = jnp.einsum("bhqk,bhkd->bhqd", p, v)
        return (lambda x, *d: x.transpose(*d))(o, 0, 2, 1, 3).reshape(B, S, D) @ wo

    def _B_ref(x, w_r, w_gate, w_up, w_down):
        B, S, D = x.shape
        C = 1
        r = x @ w_r
        idx = jnp.argsort(-r, axis=-1)[:, :C]
        idx_e = jnp.repeat(idx.reshape(B, C, 1), D, axis=2)
        x_sel = jnp.take_along_axis(x, idx_e, axis=1)
        g = _silu(x_sel @ w_gate)
        u = x_sel @ w_up
        y = (g * u) @ w_down
        r_sel = _sigmoid(jnp.take_along_axis(r, idx, axis=1))
        y = y * r_sel.reshape(B, C, 1)
        b_off = (jnp.arange(B) * S).reshape(B, 1)
        flat_idx = (idx + b_off).reshape(B * C)
        zero = (x * 0.0).reshape(B * S, D)
        upd = _scatter_add(zero, flat_idx, y.reshape(B * C, D), axis=0)
        return x + upd.reshape(B, S, D)

    x = A_x
    h = x + _A_ref(_layernorm(x, axis=-1), A_wqkv, A_wo)
    h2 = h + _B_ref(_layernorm(h, axis=-1), B_w_r, B_w_gate, B_w_up, B_w_down)
    return h2
```

```python
import functools
import math

import jax
import jax.numpy as jnp
from jax import lax
import jax.experimental.pallas as pl
import jax.experimental.pallas.tpu as pltpu

S, D, H, F = 2048, 640, 32, 1536
Dh = D // H
CQ, CK = 512, 128
NJ, NC = S // CQ, S // CK
RB = 512
NW = D // 128
EPS = 1e-5
QSCALE = math.log2(math.e) * Dh ** -0.5
NT = (((1,), (1,)), ((), ()))
TN = (((0,), (0,)), ((), ()))
f32, bf16 = jnp.float32, jnp.bfloat16


def _ln(x):
    m = jnp.mean(x, axis=-1, keepdims=True)
    xc = x - m
    v = jnp.mean(xc * xc, axis=-1, keepdims=True)
    return xc * lax.rsqrt(v + EPS)


def _store_windows(dst, rows, val):
    for w in range(NW):
        dst[w, rows, :] = val[:, 128 * w:128 * (w + 1)]
    for w in range(NW - 1):
        dst[NW + w, rows, :] = val[:, 64 + 128 * w:192 + 128 * w]


def _attention(qw_ref, kw_ref, vt_ref, ot_ref, s_c, p_c, st_c, HB):
    items = [(j, c) for j in range(NJ) for c in range(NC)]
    NI = len(items)
    lane = lax.broadcasted_iota(jnp.int32, (CQ, 128), 1)
    row8 = lax.broadcasted_iota(jnp.int32, (8, CK), 0)
    row24 = lax.broadcasted_iota(jnp.int32, (24, CK), 0)
    row24q = lax.broadcasted_iota(jnp.int32, (24, CQ), 0)
    st_m = st_c.at[pl.ds(0, 8), :]
    st_al = st_c.at[pl.ds(8, 8), :]
    st_acc = st_c.at[pl.ds(16, 24), :]

    class Head:
        def __init__(self, h, par, valid=None):
            start = h * Dh
            w = start // 128
            off = start - w * 128
            strad = off > 128 - Dh
            self.win = jnp.where(strad, w + NW, w)
            self.off = jnp.where(strad, off - 64, off)
            self.par = par
            odd = h % 2 if par is None else par
            self.odd = odd
            self.vstart = pl.multiple_of((h // 2) * 40 + odd * 16, 8)
            self.valid = valid
            self.qm = None
            self.qj = -1
            self.m = None
            self.acc = None

        def qk(self, n):
            j, c = items[n]
            if self.qj != j:
                q = qw_ref[self.win, j * CQ:(j + 1) * CQ, :]
                msk = (lane >= self.off) & (lane < self.off + Dh)
                self.qm = jnp.where(msk, q, jnp.zeros_like(q))
                self.qj = j
            kk = kw_ref[self.win, c * CK:(c + 1) * CK, :]
            return lax.dot_general(kk, self.qm, NT, preferred_element_type=f32)

        def softmax(self, n, s):
            _, c = items[n]
            cm = jnp.max(s, axis=0, keepdims=True)
            if c == 0:
                mn, al = cm, None
            else:
                mn = jnp.maximum(self.m, cm)
                al = jnp.exp2(self.m - mn)
            self.m = mn
            return jnp.exp2(s - mn).astype(bf16), al

        def pv(self, n, p, al):
            j, c = items[n]
            v = vt_ref[pl.ds(self.vstart, 24), c * CK:(c + 1) * CK]
            if self.par is None:
                v = jnp.where(row24 == jnp.where(self.odd == 1, 0, 20), 1.0, v)
            elif self.par == 0:
                v = jnp.concatenate([v[:16], jnp.where(row8 == 4, 1.0, v[16:])], axis=0)
            else:
                v = jnp.concatenate([jnp.where(row8 == 0, 1.0, v[:8]), v[8:]], axis=0)
            r = jnp.dot(v, p, preferred_element_type=f32)
            acc = r if c == 0 else self.acc * al + r
            self.acc = acc
            if c == NC - 1:
                if self.par is None:
                    l = jnp.where(self.odd == 1, acc[0:1, :], acc[20:21, :])
                else:
                    l = acc[0:1, :] if self.par == 1 else acc[20:21, :]
                o = acc * pltpu.reciprocal(l, approx=False)
                lo = self.odd * 4
                msk = (row24q >= lo) & (row24q < lo + Dh)
                if self.valid is not None:
                    msk = msk & self.valid
                pltpu.store(ot_ref.at[pl.ds(self.vstart, 24), j * CQ:(j + 1) * CQ], o, mask=msk)
                self.acc = None

    static_par = HB % 2 == 0

    def load_state(hp):
        hp.m = st_m[0:1, :]
        hp.acc = st_acc[...]
        return s_c[...], p_c[...], st_al[0:1, :]

    def body(i, carry):
        h0 = i * HB
        hp = Head(jnp.maximum(h0 - 1, 0), 1 if static_par else None, valid=(i > 0))
        heads = [Head(h0 + hh, hh % 2 if static_par else None) for hh in range(HB)]
        s_prev, p_prev, al_prev = load_state(hp)
        seq = [(hp, NI - 2), (hp, NI - 1)] + [(hd, n) for hd in heads for n in range(NI)]
        ss = {1: s_prev}
        pp = {0: (p_prev, al_prev)}
        T = len(seq)
        for t in range(2, T):
            hd, n = seq[t]
            ss[t] = hd.qk(n)
            hd1, n1 = seq[t - 1]
            pp[t - 1] = hd1.softmax(n1, ss.pop(t - 1))
            hd2, n2 = seq[t - 2]
            hd2.pv(n2, *pp.pop(t - 2))
        hd = heads[-1]
        s_c[...] = ss.pop(T - 1)
        p, al = pp.pop(T - 2)
        p_c[...] = p
        st_al[...] = jnp.broadcast_to(al, (8, CQ))
        st_m[...] = jnp.broadcast_to(hd.m, (8, CQ))
        st_acc[...] = hd.acc
        return carry

    s_c[...] = jnp.zeros(s_c.shape, f32)
    p_c[...] = jnp.zeros(p_c.shape, bf16)
    st_c[...] = jnp.ones(st_c.shape, f32)
    lax.fori_loop(0, H // HB, body, 0)
    hp = Head(H - 1, 1)
    s_prev, p_prev, al_prev = load_state(hp)
    last = hp.softmax(NI - 1, s_prev)
    hp.pv(NI - 2, p_prev, al_prev)
    hp.pv(NI - 1, *last)


def _kernel(x_hbm, wqkv_hbm, wo_hbm, wr_hbm, wg_hbm, wu_hbm, wd_hbm, out_ref,
            x_v, wqkv_v, wo_v, wr_v, wg_v, wu_v, wd_v,
            wvt_v, qw, kw, vt, ot, h_v, s_c, p_c, st_c, sems, *, HB):
    NRB = S // RB
    cp_w = pltpu.make_async_copy(wqkv_hbm, wqkv_v, sems.at[0])
    cp_x = [pltpu.make_async_copy(x_hbm.at[pl.ds(i * RB, RB), :], x_v.at[pl.ds(i * RB, RB), :], sems.at[1 + i])
            for i in range(NRB)]
    rest = [pltpu.make_async_copy(src, dst, sems.at[1 + NRB + i]) for i, (src, dst) in enumerate(
        [(wo_hbm, wo_v), (wr_hbm, wr_v), (wg_hbm, wg_v), (wu_hbm, wu_v), (wd_hbm, wd_v)])]
    cp_w.start()
    for c in cp_x:
        c.start()
    for c in rest:
        c.start()

    cp_w.wait()
    wvt_v[...] = wqkv_v[:, 2 * D:3 * D].astype(f32).T.astype(bf16)
    for i in range(NRB):
        cp_x[i].wait()
        rows = pl.ds(i * RB, RB)
        ln = _ln(x_v[rows, :].astype(f32)).astype(bf16)
        q = jnp.dot(ln, wqkv_v[:, 0:D], preferred_element_type=f32) * QSCALE
        _store_windows(qw, rows, q.astype(bf16))
        k = jnp.dot(ln, wqkv_v[:, D:2 * D], preferred_element_type=f32)
        _store_windows(kw, rows, k.astype(bf16))
        vt[:, rows] = lax.dot_general(wvt_v[...], ln, NT, preferred_element_type=f32)

    _attention(qw, kw, vt, ot, s_c, p_c, st_c, HB)

    for c in rest:
        c.wait()
    wr = wr_v[...].astype(f32)
    best = None
    for i in range(NRB):
        rows = pl.ds(i * RB, RB)
        o_t = ot[:, rows].astype(bf16)
        h = x_v[rows, :].astype(f32) + lax.dot_general(o_t, wo_v[...], TN, preferred_element_type=f32)
        h_v[rows, :] = h
        lnh = _ln(h)
        out_ref[rows, :] = (h + lnh).astype(bf16)
        r = jnp.sum(lnh.astype(bf16).astype(f32) * wr, axis=-1, keepdims=True)
        bm = jnp.max(r, axis=0, keepdims=True)
        ridx = lax.broadcasted_iota(jnp.int32, (RB, 1), 0) + i * RB
        bi = jnp.min(jnp.where(r == bm, ridx, S), axis=0, keepdims=True)
        if best is None:
            best = (bm, bi)
        else:
            take = bm > best[0]
            best = (jnp.where(take, bm, best[0]), jnp.where(take, bi, best[1]))

    rmax, ridx = best
    idx = jnp.minimum(jnp.max(ridx), S - 1)
    t0 = pl.multiple_of((idx // 16) * 16, 16)
    ht = h_v[pl.ds(t0, 16), :]
    lnt = _ln(ht)
    sel = lax.broadcasted_iota(jnp.int32, (16, D), 0) == idx - t0
    xs = jnp.sum(jnp.where(sel, lnt, 0.0), axis=0, keepdims=True)
    xs = jnp.broadcast_to(xs, (16, D)).astype(bf16)
    g = jnp.dot(xs, wg_v[...], preferred_element_type=f32)
    u = jnp.dot(xs, wu_v[...], preferred_element_type=f32)
    a = (g * jax.nn.sigmoid(g) * u).astype(bf16)
    y = jnp.dot(a, wd_v[...], preferred_element_type=f32)
    y = y * jax.nn.sigmoid(rmax)
    out_ref[pl.ds(t0, 16), :] = (ht + lnt + jnp.where(sel, y, 0.0)).astype(bf16)


def make(HB=2, name="preln_mha_mod", flags=None):
    def fn(A_x, A_wqkv, A_wo, B_x, B_w_r, B_w_gate, B_w_up, B_w_down):
        del B_x
        any_spec = pl.BlockSpec(memory_space=pl.ANY)
        out = pl.pallas_call(
            functools.partial(_kernel, HB=HB),
            in_specs=[any_spec] * 7,
            out_specs=pl.BlockSpec((S, D), lambda: (0, 0)),
            out_shape=jax.ShapeDtypeStruct((S, D), bf16),
            scratch_shapes=[
                pltpu.VMEM((S, D), bf16), pltpu.VMEM((D, 3 * D), bf16), pltpu.VMEM((D, D), bf16),
                pltpu.VMEM((1, D), bf16), pltpu.VMEM((D, F), bf16), pltpu.VMEM((D, F), bf16),
                pltpu.VMEM((F, D), bf16),
                pltpu.VMEM((D, D), bf16), pltpu.VMEM((2 * NW - 1, S, 128), bf16),
                pltpu.VMEM((2 * NW - 1, S, 128), bf16), pltpu.VMEM((D, S), f32), pltpu.VMEM((D, S), f32),
                pltpu.VMEM((S, D), f32),
                pltpu.VMEM((CK, CQ), f32), pltpu.VMEM((CK, CQ), bf16), pltpu.VMEM((40, CQ), f32),
                pltpu.SemaphoreType.DMA((10,)),
            ],
            compiler_params=pltpu.CompilerParams(vmem_limit_bytes=100 * 1024 * 1024, flags=flags),
            name=name,
        )(A_x.reshape(S, D), A_wqkv, A_wo, B_w_r.reshape(1, D), B_w_gate, B_w_up, B_w_down)
        return out.reshape(1, S, D)
    return fn


@jax.jit
def pallas_sequential_preLN__mha_block__moe_arch_mod__prompt_kernel(
    A_x: jax.Array,
    A_wqkv: jax.Array,
    A_wo: jax.Array,
    B_x: jax.Array,
    B_w_r: jax.Array,
    B_w_gate: jax.Array,
    B_w_up: jax.Array,
    B_w_down: jax.Array,
):
    return make(HB=2)(A_x, A_wqkv, A_wo, B_x, B_w_r, B_w_gate, B_w_up, B_w_down)
```

```python
import math

import jax
import jax.numpy as jnp
from jax import lax
import jax.experimental.pallas as pl
import jax.experimental.pallas.tpu as pltpu

S, D, H, F = 2048, 640, 32, 1536
Dh = D // H
NW = D // 128
CQ, CK = 512, 128
NJ, NC = S // CQ, S // CK
HB = 2
RA, SB = 512, 256
RC = 128
OUT_DMA_AFTER = (7, 14, 15)
EPS = 1e-5
QSCALE = math.log2(math.e) * Dh ** -0.5
NT = (((1,), (1,)), ((), ()))
f32, bf16 = jnp.float32, jnp.bfloat16


def _ln(x):
    xc = x - jnp.mean(x, axis=-1, keepdims=True)
    return xc * lax.rsqrt(jnp.mean(xc * xc, axis=-1, keepdims=True) + EPS)


def _pk(x):
    return pltpu.bitcast(x, jnp.int32)


def _unpk(x):
    return pltpu.bitcast(x, bf16)


def _store_shifted(dst, rows, wins):
    lane = lax.broadcasted_iota(jnp.int32, wins[0].shape, 1)
    rolled = [pltpu.roll(w, 64, 1) for w in wins]
    for w in range(NW - 1):
        dst[NW + w, rows, :] = jnp.where(lane < 64, rolled[w], rolled[w + 1])


def _store_windows(dst, r0, nr, val, shifted):
    rows = pl.ds(r0 // 2, nr // 2)
    wins = [_pk(val[:, 128 * w:128 * (w + 1)]) for w in range(NW)]
    for w in range(NW):
        dst[w, rows, :] = wins[w]
    if shifted:
        _store_shifted(dst, rows, wins)


def _attention(qw, kw, vt, ot, s_c, p_c, st_c):
    items = [(j, c) for j in range(NJ) for c in range(NC)]
    NI = len(items)
    lane = lax.broadcasted_iota(jnp.int32, (CQ // 2, 128), 1)
    row8 = lax.broadcasted_iota(jnp.int32, (8, CK), 0)
    row24 = lax.broadcasted_iota(jnp.int32, (24, CQ), 0)
    st_m = st_c.at[pl.ds(0, 8), :]
    st_acc = st_c.at[pl.ds(8, 24), :]
    st_al = st_c.at[pl.ds(32, 8), :]

    class Head:
        def __init__(self, h, odd, valid=None):
            start = h * Dh
            w = start // 128
            off = start - w * 128
            straddles = off > 128 - Dh
            self.win = jnp.where(straddles, w + NW, w)
            self.off = jnp.where(straddles, off - 64, off)
            self.odd = odd
            self.vstart = pl.multiple_of((h // 2) * 40 + odd * 16, 8)
            self.valid = valid
            self.qm, self.qj = None, -1
            self.m = self.acc = None

        def qk(self, n):
            j, c = items[n]
            if self.qj != j:
                q = qw[self.win, j * (CQ // 2):(j + 1) * (CQ // 2), :]
                mine = (lane >= self.off) & (lane < self.off + Dh)
                self.qm, self.qj = _unpk(jnp.where(mine, q, 0)), j
            k = _unpk(kw[self.win, c * (CK // 2):(c + 1) * (CK // 2), :])
            return lax.dot_general(k, self.qm, NT, preferred_element_type=f32)

        def softmax(self, n, s):
            _, c = items[n]
            cm = jnp.max(s, axis=0, keepdims=True)
            if c == 0:
                m, al = cm, None
            else:
                m = jnp.maximum(self.m, cm)
                al = jnp.exp2(self.m - m)
            self.m = m
            return jnp.exp2(s - m).astype(bf16), al

        def pv(self, n, p, al):
            j, c = items[n]
            v = vt[pl.ds(self.vstart, 24), c * CK:(c + 1) * CK]
            if self.odd:
                v = jnp.concatenate([jnp.where(row8 == 0, 1.0, v[:8]), v[8:]], axis=0)
            else:
                v = jnp.concatenate([v[:16], jnp.where(row8 == 4, 1.0, v[16:])], axis=0)
            r = jnp.dot(v, p, preferred_element_type=f32)
            self.acc = r if c == 0 else self.acc * al + r
            if c == NC - 1:
                l = self.acc[0:1, :] if self.odd else self.acc[20:21, :]
                o = self.acc * pltpu.reciprocal(l, approx=False)
                mine = row24 >= 4 if self.odd else row24 < Dh
                if self.valid is not None:
                    mine = mine & self.valid
                pltpu.store(ot.at[pl.ds(self.vstart, 24), j * CQ:(j + 1) * CQ], o, mask=mine)
                self.acc = None

    def load_state(prev):
        prev.m = st_m[0:1, :]
        prev.acc = st_acc[...]
        return s_c[...], (_unpk(p_c[...]), st_al[0:1, :])

    def body(i, carry):
        h0 = i * HB
        prev = Head(jnp.maximum(h0 - 1, 0), 1, valid=i > 0)
        heads = [Head(h0 + k, k % 2) for k in range(HB)]
        seq = [(prev, NI - 2), (prev, NI - 1)] + [(hd, n) for hd in heads for n in range(NI)]
        ss, pp = {}, {}
        ss[1], pp[0] = load_state(prev)
        for t in range(2, len(seq)):
            hd, n = seq[t]
            ss[t] = hd.qk(n)
            hd, n = seq[t - 1]
            pp[t - 1] = hd.softmax(n, ss.pop(t - 1))
            hd, n = seq[t - 2]
            hd.pv(n, *pp.pop(t - 2))
        last = heads[-1]
        s_c[...] = ss.pop(len(seq) - 1)
        p, al = pp.pop(len(seq) - 2)
        p_c[...] = _pk(p)
        st_al[...] = jnp.broadcast_to(al, (8, CQ))
        st_m[...] = jnp.broadcast_to(last.m, (8, CQ))
        st_acc[...] = last.acc
        return carry

    s_c[...] = jnp.zeros(s_c.shape, f32)
    p_c[...] = jnp.zeros(p_c.shape, jnp.int32)
    st_c[...] = jnp.ones(st_c.shape, f32)
    lax.fori_loop(0, H // HB, body, 0)
    last = Head(H - 1, 1)
    s, (p, al) = load_state(last)
    tail = last.softmax(NI - 1, s)
    last.pv(NI - 2, p, al)
    last.pv(NI - 1, *tail)


def _kernel(x_hbm, wqkv_hbm, wo_hbm, wr_hbm, wg_hbm, wu_hbm, wd_hbm, out_hbm,
            x_v, wqkv_v, wo_v, wr_v, wg_v, wu_v, wd_v,
            wvt_v, a_v, qw, kw, vt, ot, h_v, out_v, fix_v, s_c, p_c, st_c, sems, osems):
    NA, NB = S // RA, S // RC
    cp_x = [pltpu.make_async_copy(x_hbm.at[pl.ds(i * RA, RA), :], x_v.at[pl.ds(i * RA, RA), :],
                                  sems.at[i]) for i in range(NA)]
    cp_w = [pltpu.make_async_copy(wqkv_hbm.at[:, pl.ds(i * D, D)], wqkv_v.at[:, pl.ds(i * D, D)],
                                  sems.at[NA + i]) for i in range(3)]
    rest = [pltpu.make_async_copy(src, dst, sems.at[NA + 3 + i]) for i, (src, dst) in enumerate(
        [(wo_hbm, wo_v), (wr_hbm, wr_v), (wg_hbm, wg_v), (wu_hbm, wu_v), (wd_hbm, wd_v)])]
    cp_x[0].start()
    for c in cp_w:
        c.start()
    for c in cp_x[1:]:
        c.start()

    def lhs(r0, nr):
        return _unpk(a_v[r0 // 2:(r0 + nr) // 2, :])

    def do_ln(i):
        a_v[i * (RA // 2):(i + 1) * (RA // 2), :] = _pk(
            _ln(x_v[i * RA:(i + 1) * RA, :].astype(f32)).astype(bf16))

    def do_q(i, shifted=True):
        for r0 in range(i * RA, (i + 1) * RA, SB):
            q = jnp.dot(lhs(r0, SB), wqkv_v[:, 0:D], preferred_element_type=f32) * QSCALE
            _store_windows(qw, r0, SB, q.astype(bf16), shifted)

    def do_k(i, shifted=True):
        for r0 in range(i * RA, (i + 1) * RA, SB):
            k = jnp.dot(lhs(r0, SB), wqkv_v[:, D:2 * D], preferred_element_type=f32)
            _store_windows(kw, r0, SB, k.astype(bf16), shifted)

    def do_v(i):
        for r0 in range(i * RA, (i + 1) * RA, SB):
            vt[:, r0:r0 + SB] = lax.dot_general(_unpk(wvt_v[...]), lhs(r0, SB), NT,
                                                preferred_element_type=f32)

    def shift_block0(dst):
        rows = pl.ds(0, RA // 2)
        _store_shifted(dst, rows, [dst[w, rows, :] for w in range(NW)])

    cp_x[0].wait()
    do_ln(0)
    cp_w[0].wait()
    do_q(0, False)
    cp_w[1].wait()
    cp_w[2].wait()
    wvt_v[...] = _pk(wqkv_v[:, 2 * D:3 * D].T)
    do_k(0, False)
    shift_block0(qw)
    for c in cp_x[1:]:
        c.wait()
    for c in rest:
        c.start()
    do_ln(1)
    do_v(0)
    shift_block0(kw)
    for i in range(1, NA):
        do_q(i)
        if i + 1 < NA:
            do_ln(i + 1)
        do_k(i)
        do_v(i)
    for c in rest:
        c.wait()

    _attention(qw, kw, vt, ot, s_c, p_c, st_c)

    wr = wr_v[...].astype(f32).reshape(1, D)

    def transpose_o(i):
        a_v[i * (RC // 2):(i + 1) * (RC // 2), :] = _pk(ot[:, i * RC:(i + 1) * RC].astype(bf16).T)

    def project(i):
        rows = pl.ds(i * RC, RC)
        h_v[rows, :] = x_v[rows, :].astype(f32) + jnp.dot(
            lhs(i * RC, RC), wo_v[...], preferred_element_type=f32)

    def norm_and_score(i, best):
        rows = pl.ds(i * RC, RC)
        h = h_v[rows, :]
        lnh = _ln(h)
        out_v[rows, :] = (h + lnh).astype(bf16)
        r = jnp.sum(lnh.astype(bf16).astype(f32) * wr, axis=-1, keepdims=True)
        rmax = jnp.max(r, axis=0, keepdims=True)
        tok = lax.broadcasted_iota(jnp.int32, (RC, 1), 0) + i * RC
        first = jnp.min(jnp.where(r == rmax, tok, S), axis=0, keepdims=True)
        if best is None:
            return rmax, first
        take = rmax > best[0]
        return jnp.where(take, rmax, best[0]), jnp.where(take, first, best[1])

    best, sent, out_cp = None, 0, []
    transpose_o(0)
    project(0)
    for i in range(NB):
        if i + 1 < NB:
            transpose_o(i + 1)
            project(i + 1)
        best = norm_and_score(i, best)
        if i in OUT_DMA_AFTER:
            rows = pl.ds(sent * RC, (i + 1 - sent) * RC)
            out_cp.append(pltpu.make_async_copy(out_v.at[rows, :], out_hbm.at[rows, :],
                                                osems.at[len(out_cp)]))
            out_cp[-1].start()
            sent = i + 1

    rmax, tok = best
    idx = jnp.minimum(jnp.max(tok), S - 1)
    t0 = pl.multiple_of((idx // 16) * 16, 16)
    ht = h_v[pl.ds(t0, 16), :]
    lnt = _ln(ht)
    sel = lax.broadcasted_iota(jnp.int32, (16, D), 0) == idx - t0
    xs = jnp.sum(jnp.where(sel, lnt, 0.0), axis=0, keepdims=True)
    xs = jnp.broadcast_to(xs, (16, D)).astype(bf16)
    g = jnp.dot(xs, wg_v[...], preferred_element_type=f32)
    u = jnp.dot(xs, wu_v[...], preferred_element_type=f32)
    act = (g * jax.nn.sigmoid(g) * u).astype(bf16)
    y = jnp.dot(act, wd_v[...], preferred_element_type=f32) * jax.nn.sigmoid(rmax)
    fix_v[...] = (ht + lnt + jnp.where(sel, y, 0.0)).astype(bf16)
    for c in out_cp:
        c.wait()
    fix_cp = pltpu.make_async_copy(fix_v, out_hbm.at[pl.ds(t0, 16), :], osems.at[len(out_cp)])
    fix_cp.start()
    fix_cp.wait()


@jax.jit
def pallas_sequential_preLN__mha_block__moe_arch_mod__prompt_kernel(
    A_x: jax.Array,
    A_wqkv: jax.Array,
    A_wo: jax.Array,
    B_x: jax.Array,
    B_w_r: jax.Array,
    B_w_gate: jax.Array,
    B_w_up: jax.Array,
    B_w_down: jax.Array,
):
    del B_x
    hbm = pl.BlockSpec(memory_space=pl.ANY)
    out = pl.pallas_call(
        _kernel,
        in_specs=[hbm] * 7,
        out_specs=hbm,
        out_shape=jax.ShapeDtypeStruct((S, D), bf16),
        scratch_shapes=[
            pltpu.VMEM((S, D), bf16),
            pltpu.VMEM((D, 3 * D), bf16),
            pltpu.VMEM((D, D), bf16),
            pltpu.VMEM((D,), bf16),
            pltpu.VMEM((D, F), bf16),
            pltpu.VMEM((D, F), bf16),
            pltpu.VMEM((F, D), bf16),
            pltpu.VMEM((D // 2, D), jnp.int32),
            pltpu.VMEM((S // 2, D), jnp.int32),
            pltpu.VMEM((2 * NW - 1, S // 2, 128), jnp.int32),
            pltpu.VMEM((2 * NW - 1, S // 2, 128), jnp.int32),
            pltpu.VMEM((D, S), f32),
            pltpu.VMEM((D, S), f32),
            pltpu.VMEM((S, D), f32),
            pltpu.VMEM((S, D), bf16),
            pltpu.VMEM((16, D), bf16),
            pltpu.VMEM((CK, CQ), f32),
            pltpu.VMEM((CK // 2, CQ), jnp.int32),
            pltpu.VMEM((40, CQ), f32),
            pltpu.SemaphoreType.DMA((S // RA + 8,)),
            pltpu.SemaphoreType.DMA((len(OUT_DMA_AFTER) + 1,)),
        ],
        compiler_params=pltpu.CompilerParams(vmem_limit_bytes=100 * 1024 * 1024),
        name="preln_mha_mod_block",
    )(A_x.reshape(S, D), A_wqkv, A_wo, B_w_r, B_w_gate, B_w_up, B_w_down)
    return out.reshape(1, S, D)
```

```python
import math

import jax
import jax.numpy as jnp
from jax import lax
import jax.experimental.pallas as pl
import jax.experimental.pallas.tpu as pltpu

S, D, H, F = 2048, 640, 32, 1536
Dh = D // H
NW = D // 128
CQ, CK = 512, 128
NJ, NC = S // CQ, S // CK
HB = 2
RA, SB = 512, 256
RC = 128
OUT_DMA_AFTER = (7, 14, 15)
EPS = 1e-5
QSCALE = math.log2(math.e) * Dh ** -0.5
NT = (((1,), (1,)), ((), ()))
f32, bf16 = jnp.float32, jnp.bfloat16


def _ln(x):
    xc = x - jnp.mean(x, axis=-1, keepdims=True)
    return xc * lax.rsqrt(jnp.mean(xc * xc, axis=-1, keepdims=True) + EPS)


def _pk(x):
    return pltpu.bitcast(x, jnp.int32)


def _unpk(x):
    return pltpu.bitcast(x, bf16)


def _store_shifted(dst, rows, wins):
    lane = lax.broadcasted_iota(jnp.int32, wins[0].shape, 1)
    rolled = [pltpu.roll(w, 64, 1) for w in wins]
    for w in range(NW - 1):
        dst[NW + w, rows, :] = jnp.where(lane < 64, rolled[w], rolled[w + 1])


def _store_windows(dst, r0, nr, val, shifted):
    rows = pl.ds(r0 // 2, nr // 2)
    wins = [_pk(val[:, 128 * w:128 * (w + 1)]) for w in range(NW)]
    for w in range(NW):
        dst[w, rows, :] = wins[w]
    if shifted:
        _store_shifted(dst, rows, wins)


def _attention(qw, kw, vt, ot, s_c, p_c, st_c):
    items = [(j, c) for j in range(NJ) for c in range(NC)]
    NI = len(items)
    lane = lax.broadcasted_iota(jnp.int32, (CQ // 2, 128), 1)
    row8 = lax.broadcasted_iota(jnp.int32, (8, CK), 0)
    row24 = lax.broadcasted_iota(jnp.int32, (24, CQ), 0)
    st_m = st_c.at[pl.ds(0, 8), :]
    st_acc = st_c.at[pl.ds(8, 24), :]
    st_al = st_c.at[pl.ds(32, 8), :]

    class Head:
        def __init__(self, h, odd, valid=None):
            start = h * Dh
            w = start // 128
            off = start - w * 128
            straddles = off > 128 - Dh
            self.win = jnp.where(straddles, w + NW, w)
            self.off = jnp.where(straddles, off - 64, off)
            self.odd = odd
            self.vstart = pl.multiple_of((h // 2) * 40 + odd * 16, 8)
            self.valid = valid
            self.qm, self.qj = None, -1
            self.m = self.acc = None

        def qk(self, n):
            j, c = items[n]
            if self.qj != j:
                q = qw[self.win, j * (CQ // 2):(j + 1) * (CQ // 2), :]
                mine = (lane >= self.off) & (lane < self.off + Dh)
                self.qm, self.qj = _unpk(jnp.where(mine, q, 0)), j
            k = _unpk(kw[self.win, c * (CK // 2):(c + 1) * (CK // 2), :])
            return lax.dot_general(k, self.qm, NT, preferred_element_type=f32)

        def softmax(self, n, s):
            _, c = items[n]
            cm = jnp.max(s, axis=0, keepdims=True)
            if c == 0:
                m, al = cm, None
            else:
                m = jnp.maximum(self.m, cm)
                al = jnp.exp2(self.m - m)
            self.m = m
            return jnp.exp2(s - m).astype(bf16), al

        def pv(self, n, p, al):
            j, c = items[n]
            v = vt[pl.ds(self.vstart, 24), c * CK:(c + 1) * CK]
            if self.odd:
                v = jnp.concatenate([jnp.where(row8 == 0, 1.0, v[:8]), v[8:]], axis=0)
            else:
                v = jnp.concatenate([v[:16], jnp.where(row8 == 4, 1.0, v[16:])], axis=0)
            r = jnp.dot(v, p, preferred_element_type=f32)
            self.acc = r if c == 0 else self.acc * al + r
            if c == NC - 1:
                l = self.acc[0:1, :] if self.odd else self.acc[20:21, :]
                o = self.acc * pltpu.reciprocal(l, approx=False)
                mine = row24 >= 4 if self.odd else row24 < Dh
                if self.valid is not None:
                    mine = mine & self.valid
                pltpu.store(ot.at[pl.ds(self.vstart, 24), j * CQ:(j + 1) * CQ], o, mask=mine)
                self.acc = None

    def load_state(prev):
        prev.m = st_m[0:1, :]
        prev.acc = st_acc[...]
        return s_c[...], (_unpk(p_c[...]), st_al[0:1, :])

    def body(i, carry):
        h0 = i * HB
        prev = Head(jnp.maximum(h0 - 1, 0), 1, valid=i > 0)
        heads = [Head(h0 + k, k % 2) for k in range(HB)]
        seq = [(prev, NI - 2), (prev, NI - 1)] + [(hd, n) for hd in heads for n in range(NI)]
        ss, pp = {}, {}
        ss[1], pp[0] = load_state(prev)
        for t in range(2, len(seq)):
            hd, n = seq[t]
            ss[t] = hd.qk(n)
            hd, n = seq[t - 1]
            pp[t - 1] = hd.softmax(n, ss.pop(t - 1))
            hd, n = seq[t - 2]
            hd.pv(n, *pp.pop(t - 2))
        last = heads[-1]
        s_c[...] = ss.pop(len(seq) - 1)
        p, al = pp.pop(len(seq) - 2)
        p_c[...] = _pk(p)
        st_al[...] = jnp.broadcast_to(al, (8, CQ))
        st_m[...] = jnp.broadcast_to(last.m, (8, CQ))
        st_acc[...] = last.acc
        return carry

    s_c[...] = jnp.zeros(s_c.shape, f32)
    p_c[...] = jnp.zeros(p_c.shape, jnp.int32)
    st_c[...] = jnp.ones(st_c.shape, f32)
    lax.fori_loop(0, H // HB, body, 0)
    last = Head(H - 1, 1)
    s, (p, al) = load_state(last)
    tail = last.softmax(NI - 1, s)
    last.pv(NI - 2, p, al)
    last.pv(NI - 1, *tail)


def _kernel(x_hbm, wqkv_hbm, wo_hbm, wr_hbm, wg_hbm, wu_hbm, wd_hbm, out_hbm,
            x_v, wqkv_v, wo_v, wr_v, wg_v, wu_v, wd_v,
            wvt_v, a_v, qw, kw, vt, ot, h_v, out_v, fix_v, s_c, p_c, st_c, sems, osems):
    NA, NB = S // RA, S // RC
    cp_x = [pltpu.make_async_copy(x_hbm.at[pl.ds(i * RA, RA), :], x_v.at[pl.ds(i * RA, RA), :],
                                  sems.at[i]) for i in range(NA)]
    cp_w = [pltpu.make_async_copy(wqkv_hbm.at[:, pl.ds(i * D, D)], wqkv_v.at[:, pl.ds(i * D, D)],
                                  sems.at[NA + i]) for i in range(3)]
    rest = [pltpu.make_async_copy(src, dst, sems.at[NA + 3 + i]) for i, (src, dst) in enumerate(
        [(wo_hbm, wo_v), (wr_hbm, wr_v), (wg_hbm, wg_v), (wu_hbm, wu_v), (wd_hbm, wd_v)])]
    for c in (cp_x[0], cp_w[0], cp_w[1], cp_x[1], cp_w[2], cp_x[2], cp_x[3]):
        c.start()

    def lhs(r0, nr):
        return _unpk(a_v[r0 // 2:(r0 + nr) // 2, :])

    def do_ln(i):
        a_v[i * (RA // 2):(i + 1) * (RA // 2), :] = _pk(
            _ln(x_v[i * RA:(i + 1) * RA, :].astype(f32)).astype(bf16))

    def do_q(i, shifted=True):
        for r0 in range(i * RA, (i + 1) * RA, SB):
            q = jnp.dot(lhs(r0, SB), wqkv_v[:, 0:D], preferred_element_type=f32) * QSCALE
            _store_windows(qw, r0, SB, q.astype(bf16), shifted)

    def shift_q(i):
        rows = pl.ds(i * (RA // 2), RA // 2)
        _store_shifted(qw, rows, [qw[w, rows, :] for w in range(NW)])

    def do_k(i):
        for r0 in range(i * RA, (i + 1) * RA, SB):
            k = jnp.dot(lhs(r0, SB), wqkv_v[:, D:2 * D], preferred_element_type=f32)
            _store_windows(kw, r0, SB, k.astype(bf16), True)

    def do_v(i):
        for r0 in range(i * RA, (i + 1) * RA, SB):
            vt[:, r0:r0 + SB] = lax.dot_general(_unpk(wvt_v[...]), lhs(r0, SB), NT,
                                                preferred_element_type=f32)

    cp_x[0].wait()
    do_ln(0)
    cp_w[0].wait()
    do_q(0, False)
    cp_w[1].wait()
    cp_x[1].wait()
    do_ln(1)
    do_k(0)
    shift_q(0)
    do_q(1, False)
    cp_w[2].wait()
    cp_x[2].wait()
    cp_x[3].wait()
    for c in rest:
        c.start()
    wvt_v[...] = _pk(wqkv_v[:, 2 * D:3 * D].T)
    do_k(1)
    do_ln(2)
    shift_q(1)
    do_v(0)
    do_v(1)
    for i in range(2, NA):
        do_q(i)
        if i + 1 < NA:
            do_ln(i + 1)
        do_k(i)
        do_v(i)
    for c in rest:
        c.wait()

    _attention(qw, kw, vt, ot, s_c, p_c, st_c)

    wr = wr_v[...].astype(f32).reshape(1, D)

    def transpose_o(i):
        a_v[i * (RC // 2):(i + 1) * (RC // 2), :] = _pk(ot[:, i * RC:(i + 1) * RC].astype(bf16).T)

    def project(i):
        rows = pl.ds(i * RC, RC)
        h_v[rows, :] = x_v[rows, :].astype(f32) + jnp.dot(
            lhs(i * RC, RC), wo_v[...], preferred_element_type=f32)

    def norm_and_score(i, best):
        rows = pl.ds(i * RC, RC)
        h = h_v[rows, :]
        lnh = _ln(h)
        out_v[rows, :] = (h + lnh).astype(bf16)
        r = jnp.sum(lnh.astype(bf16).astype(f32) * wr, axis=-1, keepdims=True)
        rmax = jnp.max(r, axis=0, keepdims=True)
        tok = lax.broadcasted_iota(jnp.int32, (RC, 1), 0) + i * RC
        first = jnp.min(jnp.where(r == rmax, tok, S), axis=0, keepdims=True)
        if best is None:
            return rmax, first
        take = rmax > best[0]
        return jnp.where(take, rmax, best[0]), jnp.where(take, first, best[1])

    best, sent, out_cp = None, 0, []
    transpose_o(0)
    project(0)
    for i in range(NB):
        if i + 1 < NB:
            transpose_o(i + 1)
            project(i + 1)
        best = norm_and_score(i, best)
        if i in OUT_DMA_AFTER:
            rows = pl.ds(sent * RC, (i + 1 - sent) * RC)
            out_cp.append(pltpu.make_async_copy(out_v.at[rows, :], out_hbm.at[rows, :],
                                                osems.at[len(out_cp)]))
            out_cp[-1].start()
            sent = i + 1

    rmax, tok = best
    idx = jnp.minimum(jnp.max(tok), S - 1)
    t0 = pl.multiple_of((idx // 16) * 16, 16)
    ht = h_v[pl.ds(t0, 16), :]
    lnt = _ln(ht)
    sel = lax.broadcasted_iota(jnp.int32, (16, D), 0) == idx - t0
    xs = jnp.sum(jnp.where(sel, lnt, 0.0), axis=0, keepdims=True)
    xs = jnp.broadcast_to(xs, (16, D)).astype(bf16)
    g = jnp.dot(xs, wg_v[...], preferred_element_type=f32)
    u = jnp.dot(xs, wu_v[...], preferred_element_type=f32)
    act = (g * jax.nn.sigmoid(g) * u).astype(bf16)
    y = jnp.dot(act, wd_v[...], preferred_element_type=f32) * jax.nn.sigmoid(rmax)
    fix_v[...] = (ht + lnt + jnp.where(sel, y, 0.0)).astype(bf16)
    for c in out_cp:
        c.wait()
    fix_cp = pltpu.make_async_copy(fix_v, out_hbm.at[pl.ds(t0, 16), :], osems.at[len(out_cp)])
    fix_cp.start()
    fix_cp.wait()


@jax.jit
def pallas_sequential_preLN__mha_block__moe_arch_mod__prompt_kernel(
    A_x: jax.Array,
    A_wqkv: jax.Array,
    A_wo: jax.Array,
    B_x: jax.Array,
    B_w_r: jax.Array,
    B_w_gate: jax.Array,
    B_w_up: jax.Array,
    B_w_down: jax.Array,
):
    del B_x
    hbm = pl.BlockSpec(memory_space=pl.ANY)
    out = pl.pallas_call(
        _kernel,
        in_specs=[hbm] * 7,
        out_specs=hbm,
        out_shape=jax.ShapeDtypeStruct((S, D), bf16),
        scratch_shapes=[
            pltpu.VMEM((S, D), bf16),
            pltpu.VMEM((D, 3 * D), bf16),
            pltpu.VMEM((D, D), bf16),
            pltpu.VMEM((D,), bf16),
            pltpu.VMEM((D, F), bf16),
            pltpu.VMEM((D, F), bf16),
            pltpu.VMEM((F, D), bf16),
            pltpu.VMEM((D // 2, D), jnp.int32),
            pltpu.VMEM((S // 2, D), jnp.int32),
            pltpu.VMEM((2 * NW - 1, S // 2, 128), jnp.int32),
            pltpu.VMEM((2 * NW - 1, S // 2, 128), jnp.int32),
            pltpu.VMEM((D, S), f32),
            pltpu.VMEM((D, S), f32),
            pltpu.VMEM((S, D), f32),
            pltpu.VMEM((S, D), bf16),
            pltpu.VMEM((16, D), bf16),
            pltpu.VMEM((CK, CQ), f32),
            pltpu.VMEM((CK // 2, CQ), jnp.int32),
            pltpu.VMEM((40, CQ), f32),
            pltpu.SemaphoreType.DMA((S // RA + 8,)),
            pltpu.SemaphoreType.DMA((len(OUT_DMA_AFTER) + 1,)),
        ],
        compiler_params=pltpu.CompilerParams(vmem_limit_bytes=100 * 1024 * 1024),
        name="preln_mha_mod_block",
    )(A_x.reshape(S, D), A_wqkv, A_wo, B_w_r, B_w_gate, B_w_up, B_w_down)
    return out.reshape(1, S, D)
```

```python
import math

import jax
import jax.numpy as jnp
from jax import lax
import jax.experimental.pallas as pl
import jax.experimental.pallas.tpu as pltpu

S, D, H, F = 2048, 640, 32, 1536
Dh = D // H
NW = D // 128
CQ, CK = 512, 128
NJ, NC = S // CQ, S // CK
HB = 2
RA, SB = 512, 256
RC = 128
OUT_DMA_AFTER = (7, 14, 15)
EPS = 1e-5
QSCALE = math.log2(math.e) * Dh ** -0.5
NT = (((1,), (1,)), ((), ()))
f32, bf16 = jnp.float32, jnp.bfloat16


def _ln(x):
    xc = x - jnp.mean(x, axis=-1, keepdims=True)
    return xc * lax.rsqrt(jnp.mean(xc * xc, axis=-1, keepdims=True) + EPS)


def _pk(x):
    return pltpu.bitcast(x, jnp.int32)


def _unpk(x):
    return pltpu.bitcast(x, bf16)


def _store_shifted(dst, rows, wins):
    lane = lax.broadcasted_iota(jnp.int32, wins[0].shape, 1)
    rolled = [pltpu.roll(w, 64, 1) for w in wins]
    for w in range(NW - 1):
        dst[NW + w, rows, :] = jnp.where(lane < 64, rolled[w], rolled[w + 1])


def _store_windows(dst, r0, nr, val, shifted):
    rows = pl.ds(r0 // 2, nr // 2)
    wins = [_pk(val[:, 128 * w:128 * (w + 1)]) for w in range(NW)]
    for w in range(NW):
        dst[w, rows, :] = wins[w]
    if shifted:
        _store_shifted(dst, rows, wins)


def _attention(qw, kw, vt, ot, s_c, p_c, st_c, q_c):
    items = [(j, c) for j in range(NJ) for c in range(NC)]
    NI = len(items)
    lane = lax.broadcasted_iota(jnp.int32, (CQ // 2, 128), 1)
    row8 = lax.broadcasted_iota(jnp.int32, (8, CK), 0)
    row24 = lax.broadcasted_iota(jnp.int32, (24, CQ), 0)
    st_m = st_c.at[pl.ds(0, 8), :]
    st_acc = st_c.at[pl.ds(8, 24), :]
    st_al = st_c.at[pl.ds(32, 8), :]

    class Head:
        def __init__(self, h, odd, valid=None):
            start = h * Dh
            w = start // 128
            off = start - w * 128
            straddles = off > 128 - Dh
            self.win = jnp.where(straddles, w + NW, w)
            self.off = jnp.where(straddles, off - 64, off)
            self.odd = odd
            self.vstart = pl.multiple_of((h // 2) * 40 + odd * 16, 8)
            self.valid = valid
            self.first = False
            self.qm, self.qj = None, -1
            self.m = self.acc = None

        def masked_q(self, j):
            q = qw[self.win, j * (CQ // 2):(j + 1) * (CQ // 2), :]
            mine = (lane >= self.off) & (lane < self.off + Dh)
            return jnp.where(mine, q, 0)

        def qk(self, n):
            j, c = items[n]
            if self.qj != j:
                self.qm, self.qj = _unpk(q_c[...] if (self.first and j == 0) else self.masked_q(j)), j
            k = _unpk(kw[self.win, c * (CK // 2):(c + 1) * (CK // 2), :])
            return lax.dot_general(k, self.qm, NT, preferred_element_type=f32)

        def softmax(self, n, s):
            _, c = items[n]
            cm = jnp.max(s, axis=0, keepdims=True)
            if c == 0:
                m, al = cm, None
            else:
                m = jnp.maximum(self.m, cm)
                al = jnp.exp2(self.m - m)
            self.m = m
            return jnp.exp2(s - m).astype(bf16), al

        def pv(self, n, p, al):
            j, c = items[n]
            v = vt[pl.ds(self.vstart, 24), c * CK:(c + 1) * CK]
            if self.odd:
                v = jnp.concatenate([jnp.where(row8 == 0, 1.0, v[:8]), v[8:]], axis=0)
            else:
                v = jnp.concatenate([v[:16], jnp.where(row8 == 4, 1.0, v[16:])], axis=0)
            r = jnp.dot(v, p, preferred_element_type=f32)
            self.acc = r if c == 0 else self.acc * al + r
            if c == NC - 1:
                l = self.acc[0:1, :] if self.odd else self.acc[20:21, :]
                o = self.acc * pltpu.reciprocal(l, approx=False)
                mine = row24 >= 4 if self.odd else row24 < Dh
                if self.valid is not None:
                    mine = mine & self.valid
                pltpu.store(ot.at[pl.ds(self.vstart, 24), j * CQ:(j + 1) * CQ], o, mask=mine)
                self.acc = None

    def load_state(prev):
        prev.m = st_m[0:1, :]
        prev.acc = st_acc[...]
        return s_c[...], (_unpk(p_c[...]), st_al[0:1, :])

    def body(i, carry):
        h0 = i * HB
        prev = Head(jnp.maximum(h0 - 1, 0), 1, valid=i > 0)
        heads = [Head(h0 + k, k % 2) for k in range(HB)]
        heads[0].first = True
        seq = [(prev, NI - 2), (prev, NI - 1)] + [(hd, n) for hd in heads for n in range(NI)]
        ss, pp = {}, {}
        ss[1], pp[0] = load_state(prev)
        for t in range(2, len(seq)):
            if t == 2:
                prev.pv(NI - 2, *pp.pop(0))
            hd, n = seq[t]
            ss[t] = hd.qk(n)
            hd, n = seq[t - 1]
            pp[t - 1] = hd.softmax(n, ss.pop(t - 1))
            if t > 2:
                hd, n = seq[t - 2]
                hd.pv(n, *pp.pop(t - 2))
        last = heads[-1]
        s_c[...] = ss.pop(len(seq) - 1)
        p, al = pp.pop(len(seq) - 2)
        p_c[...] = _pk(p)
        st_al[...] = jnp.broadcast_to(al, (8, CQ))
        st_m[...] = jnp.broadcast_to(last.m, (8, CQ))
        st_acc[...] = last.acc
        q_c[...] = Head(jnp.minimum(h0 + HB, H - 1), 0).masked_q(0)
        return carry

    s_c[...] = jnp.zeros(s_c.shape, f32)
    p_c[...] = jnp.zeros(p_c.shape, jnp.int32)
    st_c[...] = jnp.ones(st_c.shape, f32)
    q_c[...] = Head(0, 0).masked_q(0)
    lax.fori_loop(0, H // HB, body, 0)
    last = Head(H - 1, 1)
    s, (p, al) = load_state(last)
    tail = last.softmax(NI - 1, s)
    last.pv(NI - 2, p, al)
    last.pv(NI - 1, *tail)


def _kernel(x_hbm, wqkv_hbm, wo_hbm, wr_hbm, wg_hbm, wu_hbm, wd_hbm, out_hbm,
            x_v, wqkv_v, wo_v, wr_v, wg_v, wu_v, wd_v,
            wvt_v, a_v, qw, kw, vt, ot, h_v, out_v, fix_v, s_c, p_c, st_c, q_c, sems, osems):
    NA, NB = S // RA, S // RC
    cp_x = [pltpu.make_async_copy(x_hbm.at[pl.ds(i * RA, RA), :], x_v.at[pl.ds(i * RA, RA), :],
                                  sems.at[i]) for i in range(NA)]
    cp_w = [pltpu.make_async_copy(wqkv_hbm.at[:, pl.ds(i * D, D)], wqkv_v.at[:, pl.ds(i * D, D)],
                                  sems.at[NA + i]) for i in range(3)]
    rest = [pltpu.make_async_copy(src, dst, sems.at[NA + 3 + i]) for i, (src, dst) in enumerate(
        [(wo_hbm, wo_v), (wr_hbm, wr_v), (wg_hbm, wg_v), (wu_hbm, wu_v), (wd_hbm, wd_v)])]
    for c in (cp_x[0], cp_w[0], cp_w[1], cp_x[1], cp_w[2], cp_x[2], cp_x[3]):
        c.start()

    def lhs(r0, nr):
        return _unpk(a_v[r0 // 2:(r0 + nr) // 2, :])

    def do_ln(i):
        a_v[i * (RA // 2):(i + 1) * (RA // 2), :] = _pk(
            _ln(x_v[i * RA:(i + 1) * RA, :].astype(f32)).astype(bf16))

    def do_q(i, shifted=True):
        for r0 in range(i * RA, (i + 1) * RA, SB):
            q = jnp.dot(lhs(r0, SB), wqkv_v[:, 0:D], preferred_element_type=f32) * QSCALE
            _store_windows(qw, r0, SB, q.astype(bf16), shifted)

    def shift_q(i):
        rows = pl.ds(i * (RA // 2), RA // 2)
        _store_shifted(qw, rows, [qw[w, rows, :] for w in range(NW)])

    def do_k(i):
        for r0 in range(i * RA, (i + 1) * RA, SB):
            k = jnp.dot(lhs(r0, SB), wqkv_v[:, D:2 * D], preferred_element_type=f32)
            _store_windows(kw, r0, SB, k.astype(bf16), True)

    def do_v(i):
        for r0 in range(i * RA, (i + 1) * RA, SB):
            vt[:, r0:r0 + SB] = lax.dot_general(_unpk(wvt_v[...]), lhs(r0, SB), NT,
                                                preferred_element_type=f32)

    cp_x[0].wait()
    do_ln(0)
    cp_w[0].wait()
    do_q(0, False)
    cp_w[1].wait()
    cp_x[1].wait()
    do_ln(1)
    do_k(0)
    shift_q(0)
    do_q(1, False)
    cp_w[2].wait()
    cp_x[2].wait()
    cp_x[3].wait()
    for c in rest:
        c.start()
    wvt_v[...] = _pk(wqkv_v[:, 2 * D:3 * D].T)
    do_k(1)
    do_ln(2)
    shift_q(1)
    do_v(0)
    do_v(1)
    for i in range(2, NA):
        do_q(i)
        if i + 1 < NA:
            do_ln(i + 1)
        do_k(i)
        do_v(i)
    for c in rest:
        c.wait()

    _attention(qw, kw, vt, ot, s_c, p_c, st_c, q_c)

    wr = wr_v[...].astype(f32).reshape(1, D)

    def transpose_o(i):
        a_v[i * (RC // 2):(i + 1) * (RC // 2), :] = _pk(ot[:, i * RC:(i + 1) * RC].astype(bf16).T)

    def project(i):
        rows = pl.ds(i * RC, RC)
        h_v[rows, :] = x_v[rows, :].astype(f32) + jnp.dot(
            lhs(i * RC, RC), wo_v[...], preferred_element_type=f32)

    def norm_and_score(i, best):
        rows = pl.ds(i * RC, RC)
        h = h_v[rows, :]
        lnh = _ln(h)
        out_v[rows, :] = (h + lnh).astype(bf16)
        r = jnp.sum(lnh.astype(bf16).astype(f32) * wr, axis=-1, keepdims=True)
        rmax = jnp.max(r, axis=0, keepdims=True)
        tok = lax.broadcasted_iota(jnp.int32, (RC, 1), 0) + i * RC
        first = jnp.min(jnp.where(r == rmax, tok, S), axis=0, keepdims=True)
        if best is None:
            return rmax, first
        take = rmax > best[0]
        return jnp.where(take, rmax, best[0]), jnp.where(take, first, best[1])

    best, sent, out_cp = None, 0, []
    transpose_o(0)
    project(0)
    for i in range(NB):
        if i + 1 < NB:
            transpose_o(i + 1)
            project(i + 1)
        best = norm_and_score(i, best)
        if i in OUT_DMA_AFTER:
            rows = pl.ds(sent * RC, (i + 1 - sent) * RC)
            out_cp.append(pltpu.make_async_copy(out_v.at[rows, :], out_hbm.at[rows, :],
                                                osems.at[len(out_cp)]))
            out_cp[-1].start()
            sent = i + 1

    rmax, tok = best
    idx = jnp.minimum(jnp.max(tok), S - 1)
    t0 = pl.multiple_of((idx // 16) * 16, 16)
    ht = h_v[pl.ds(t0, 16), :]
    lnt = _ln(ht)
    sel = lax.broadcasted_iota(jnp.int32, (16, D), 0) == idx - t0
    xs = jnp.sum(jnp.where(sel, lnt, 0.0), axis=0, keepdims=True)
    xs = jnp.broadcast_to(xs, (16, D)).astype(bf16)
    g = jnp.dot(xs, wg_v[...], preferred_element_type=f32)
    u = jnp.dot(xs, wu_v[...], preferred_element_type=f32)
    act = (g * jax.nn.sigmoid(g) * u).astype(bf16)
    y = jnp.dot(act, wd_v[...], preferred_element_type=f32) * jax.nn.sigmoid(rmax)
    fix_v[...] = (ht + lnt + jnp.where(sel, y, 0.0)).astype(bf16)
    for c in out_cp:
        c.wait()
    fix_cp = pltpu.make_async_copy(fix_v, out_hbm.at[pl.ds(t0, 16), :], osems.at[len(out_cp)])
    fix_cp.start()
    fix_cp.wait()


@jax.jit
def pallas_sequential_preLN__mha_block__moe_arch_mod__prompt_kernel(
    A_x: jax.Array,
    A_wqkv: jax.Array,
    A_wo: jax.Array,
    B_x: jax.Array,
    B_w_r: jax.Array,
    B_w_gate: jax.Array,
    B_w_up: jax.Array,
    B_w_down: jax.Array,
):
    del B_x
    hbm = pl.BlockSpec(memory_space=pl.ANY)
    out = pl.pallas_call(
        _kernel,
        in_specs=[hbm] * 7,
        out_specs=hbm,
        out_shape=jax.ShapeDtypeStruct((S, D), bf16),
        scratch_shapes=[
            pltpu.VMEM((S, D), bf16),
            pltpu.VMEM((D, 3 * D), bf16),
            pltpu.VMEM((D, D), bf16),
            pltpu.VMEM((D,), bf16),
            pltpu.VMEM((D, F), bf16),
            pltpu.VMEM((D, F), bf16),
            pltpu.VMEM((F, D), bf16),
            pltpu.VMEM((D // 2, D), jnp.int32),
            pltpu.VMEM((S // 2, D), jnp.int32),
            pltpu.VMEM((2 * NW - 1, S // 2, 128), jnp.int32),
            pltpu.VMEM((2 * NW - 1, S // 2, 128), jnp.int32),
            pltpu.VMEM((D, S), f32),
            pltpu.VMEM((D, S), f32),
            pltpu.VMEM((S, D), f32),
            pltpu.VMEM((S, D), bf16),
            pltpu.VMEM((16, D), bf16),
            pltpu.VMEM((CK, CQ), f32),
            pltpu.VMEM((CK // 2, CQ), jnp.int32),
            pltpu.VMEM((40, CQ), f32),
            pltpu.VMEM((CQ // 2, 128), jnp.int32),
            pltpu.SemaphoreType.DMA((S // RA + 8,)),
            pltpu.SemaphoreType.DMA((len(OUT_DMA_AFTER) + 1,)),
        ],
        compiler_params=pltpu.CompilerParams(vmem_limit_bytes=100 * 1024 * 1024),
        name="preln_mha_mod_block",
    )(A_x.reshape(S, D), A_wqkv, A_wo, B_w_r, B_w_gate, B_w_up, B_w_down)
    return out.reshape(1, S, D)
```

```python
import math

import jax
import jax.numpy as jnp
from jax import lax
import jax.experimental.pallas as pl
import jax.experimental.pallas.tpu as pltpu

S, D, H, F = 2048, 640, 32, 1536
Dh = D // H
NW = D // 128
CQ, CK = 512, 128
NJ, NC = S // CQ, S // CK
HB = 2
RA, SB = 512, 256
RC = 128
OUT_DMA_AFTER = (7, 14, 15)
EPS = 1e-5
EPS_BF16 = 1.0013580322265625e-05
QSCALE = math.log2(math.e) * Dh ** -0.5
NT = (((1,), (1,)), ((), ()))
f32, bf16 = jnp.float32, jnp.bfloat16


def _ln(x):
    xc = x - jnp.mean(x, axis=-1, keepdims=True)
    return xc * lax.rsqrt(jnp.mean(xc * xc, axis=-1, keepdims=True) + EPS)


def _rb(x):
    return x.astype(bf16).astype(f32)


def _ln_bf16(x):
    mean = jnp.mean(x, axis=-1, keepdims=True)
    mean_b = _rb(mean)
    xc = x - mean_b
    var = jnp.mean(xc * xc, axis=-1, keepdims=True) - (mean - mean_b) * (mean - mean_b)
    sd = _rb(jnp.sqrt(_rb(_rb(var) + EPS_BF16)))
    return (_rb(xc) * pltpu.reciprocal(sd, approx=False)).astype(bf16)


def _pk(x):
    return pltpu.bitcast(x, jnp.int32)


def _unpk(x):
    return pltpu.bitcast(x, bf16)


def _store_shifted(dst, rows, wins):
    lane = lax.broadcasted_iota(jnp.int32, wins[0].shape, 1)
    rolled = [pltpu.roll(w, 64, 1) for w in wins]
    for w in range(NW - 1):
        dst[NW + w, rows, :] = jnp.where(lane < 64, rolled[w], rolled[w + 1])


def _store_windows(dst, r0, nr, val, shifted):
    rows = pl.ds(r0 // 2, nr // 2)
    wins = [_pk(val[:, 128 * w:128 * (w + 1)]) for w in range(NW)]
    for w in range(NW):
        dst[w, rows, :] = wins[w]
    if shifted:
        _store_shifted(dst, rows, wins)


def _attention(qw, kw, vt, ot, s_c, p_c, st_c, q_c):
    items = [(j, c) for j in range(NJ) for c in range(NC)]
    NI = len(items)
    lane = lax.broadcasted_iota(jnp.int32, (CQ // 2, 128), 1)
    row8 = lax.broadcasted_iota(jnp.int32, (8, CK), 0)
    row24 = lax.broadcasted_iota(jnp.int32, (24, CQ), 0)
    st_m = st_c.at[pl.ds(0, 8), :]
    st_acc = st_c.at[pl.ds(8, 24), :]
    st_al = st_c.at[pl.ds(32, 8), :]

    class Head:
        def __init__(self, h, odd, valid=None):
            start = h * Dh
            w = start // 128
            off = start - w * 128
            straddles = off > 128 - Dh
            self.win = jnp.where(straddles, w + NW, w)
            self.off = jnp.where(straddles, off - 64, off)
            self.odd = odd
            self.vstart = pl.multiple_of((h // 2) * 40 + odd * 16, 8)
            self.valid = valid
            self.first = False
            self.qm, self.qj = None, -1
            self.m = self.acc = None

        def masked_q(self, j):
            q = qw[self.win, j * (CQ // 2):(j + 1) * (CQ // 2), :]
            mine = (lane >= self.off) & (lane < self.off + Dh)
            return jnp.where(mine, q, 0)

        def qk(self, n):
            j, c = items[n]
            if self.qj != j:
                self.qm, self.qj = _unpk(q_c[...] if (self.first and j == 0) else self.masked_q(j)), j
            k = _unpk(kw[self.win, c * (CK // 2):(c + 1) * (CK // 2), :])
            return lax.dot_general(k, self.qm, NT, preferred_element_type=f32)

        def softmax(self, n, s):
            _, c = items[n]
            cm = jnp.max(s, axis=0, keepdims=True)
            if c == 0:
                m, al = cm, None
            else:
                m = jnp.maximum(self.m, cm)
                al = jnp.exp2(self.m - m)
            self.m = m
            return jnp.exp2(s - m).astype(bf16), al

        def pv(self, n, p, al):
            j, c = items[n]
            v = vt[pl.ds(self.vstart, 24), c * CK:(c + 1) * CK]
            if self.odd:
                v = jnp.concatenate([jnp.where(row8 == 0, 1.0, v[:8]), v[8:]], axis=0)
            else:
                v = jnp.concatenate([v[:16], jnp.where(row8 == 4, 1.0, v[16:])], axis=0)
            r = jnp.dot(v, p, preferred_element_type=f32)
            self.acc = r if c == 0 else self.acc * al + r
            if c == NC - 1:
                l = self.acc[0:1, :] if self.odd else self.acc[20:21, :]
                o = self.acc * pltpu.reciprocal(l, approx=False)
                mine = row24 >= 4 if self.odd else row24 < Dh
                if self.valid is not None:
                    mine = mine & self.valid
                pltpu.store(ot.at[pl.ds(self.vstart, 24), j * CQ:(j + 1) * CQ], o, mask=mine)
                self.acc = None

    def load_state(prev):
        prev.m = st_m[0:1, :]
        prev.acc = st_acc[...]
        return s_c[...], (_unpk(p_c[...]), st_al[0:1, :])

    def body(i, carry):
        h0 = i * HB
        prev = Head(jnp.maximum(h0 - 1, 0), 1, valid=i > 0)
        heads = [Head(h0 + k, k % 2) for k in range(HB)]
        heads[0].first = True
        seq = [(prev, NI - 2), (prev, NI - 1)] + [(hd, n) for hd in heads for n in range(NI)]
        ss, pp = {}, {}
        ss[1], pp[0] = load_state(prev)
        for t in range(2, len(seq)):
            if t == 2:
                prev.pv(NI - 2, *pp.pop(0))
            hd, n = seq[t]
            ss[t] = hd.qk(n)
            hd, n = seq[t - 1]
            pp[t - 1] = hd.softmax(n, ss.pop(t - 1))
            if t > 2:
                hd, n = seq[t - 2]
                hd.pv(n, *pp.pop(t - 2))
        last = heads[-1]
        s_c[...] = ss.pop(len(seq) - 1)
        p, al = pp.pop(len(seq) - 2)
        p_c[...] = _pk(p)
        st_al[...] = jnp.broadcast_to(al, (8, CQ))
        st_m[...] = jnp.broadcast_to(last.m, (8, CQ))
        st_acc[...] = last.acc
        q_c[...] = Head(jnp.minimum(h0 + HB, H - 1), 0).masked_q(0)
        return carry

    s_c[...] = jnp.zeros(s_c.shape, f32)
    p_c[...] = jnp.zeros(p_c.shape, jnp.int32)
    st_c[...] = jnp.ones(st_c.shape, f32)
    q_c[...] = Head(0, 0).masked_q(0)
    lax.fori_loop(0, H // HB, body, 0)
    last = Head(H - 1, 1)
    s, (p, al) = load_state(last)
    tail = last.softmax(NI - 1, s)
    last.pv(NI - 2, p, al)
    last.pv(NI - 1, *tail)


def _kernel(x_hbm, wqkv_hbm, wo_hbm, wr_hbm, wg_hbm, wu_hbm, wd_hbm, out_hbm,
            x_v, wqkv_v, wo_v, wr_v, wg_v, wu_v, wd_v,
            wvt_v, a_v, qw, kw, vt, ot, h_v, out_v, fix_v, s_c, p_c, st_c, q_c, sems, osems):
    NA, NB = S // RA, S // RC
    cp_x = [pltpu.make_async_copy(x_hbm.at[pl.ds(i * RA, RA), :], x_v.at[pl.ds(i * RA, RA), :],
                                  sems.at[i]) for i in range(NA)]
    cp_w = [pltpu.make_async_copy(wqkv_hbm.at[:, pl.ds(i * D, D)], wqkv_v.at[:, pl.ds(i * D, D)],
                                  sems.at[NA + i]) for i in range(3)]
    rest = [pltpu.make_async_copy(src, dst, sems.at[NA + 3 + i]) for i, (src, dst) in enumerate(
        [(wo_hbm, wo_v), (wr_hbm, wr_v), (wg_hbm, wg_v), (wu_hbm, wu_v), (wd_hbm, wd_v)])]
    for c in (cp_x[0], cp_w[0], cp_w[1], cp_x[1], cp_w[2], cp_x[2], cp_x[3]):
        c.start()

    def lhs(r0, nr):
        return _unpk(a_v[r0 // 2:(r0 + nr) // 2, :])

    def do_ln(i):
        a_v[i * (RA // 2):(i + 1) * (RA // 2), :] = _pk(_ln_bf16(x_v[i * RA:(i + 1) * RA, :].astype(f32)))

    def do_q(i, shifted=True):
        for r0 in range(i * RA, (i + 1) * RA, SB):
            q = jnp.dot(lhs(r0, SB), wqkv_v[:, 0:D], preferred_element_type=f32) * QSCALE
            _store_windows(qw, r0, SB, q.astype(bf16), shifted)

    def shift_q(i):
        rows = pl.ds(i * (RA // 2), RA // 2)
        _store_shifted(qw, rows, [qw[w, rows, :] for w in range(NW)])

    def do_k(i):
        for r0 in range(i * RA, (i + 1) * RA, SB):
            k = jnp.dot(lhs(r0, SB), wqkv_v[:, D:2 * D], preferred_element_type=f32)
            _store_windows(kw, r0, SB, k.astype(bf16), True)

    def do_v(i):
        for r0 in range(i * RA, (i + 1) * RA, SB):
            vt[:, r0:r0 + SB] = lax.dot_general(_unpk(wvt_v[...]), lhs(r0, SB), NT,
                                                preferred_element_type=f32)

    cp_x[0].wait()
    do_ln(0)
    cp_w[0].wait()
    do_q(0, False)
    cp_w[1].wait()
    cp_x[1].wait()
    do_ln(1)
    do_k(0)
    shift_q(0)
    do_q(1, False)
    cp_w[2].wait()
    cp_x[2].wait()
    cp_x[3].wait()
    for c in rest:
        c.start()
    wvt_v[...] = _pk(wqkv_v[:, 2 * D:3 * D].T)
    do_k(1)
    do_ln(2)
    shift_q(1)
    do_v(0)
    do_v(1)
    for i in range(2, NA):
        do_q(i)
        if i + 1 < NA:
            do_ln(i + 1)
        do_k(i)
        do_v(i)
    for c in rest:
        c.wait()

    _attention(qw, kw, vt, ot, s_c, p_c, st_c, q_c)

    wr = wr_v[...].astype(f32).reshape(1, D)

    def transpose_o(i):
        a_v[i * (RC // 2):(i + 1) * (RC // 2), :] = _pk(ot[:, i * RC:(i + 1) * RC].astype(bf16).T)

    def project(i):
        rows = pl.ds(i * RC, RC)
        h_v[rows, :] = x_v[rows, :].astype(f32) + jnp.dot(
            lhs(i * RC, RC), wo_v[...], preferred_element_type=f32)

    def norm_and_score(i, best):
        rows = pl.ds(i * RC, RC)
        h = h_v[rows, :]
        lnh = _ln(h)
        out_v[rows, :] = (h + lnh).astype(bf16)
        r = jnp.sum(lnh.astype(bf16).astype(f32) * wr, axis=-1, keepdims=True)
        rmax = jnp.max(r, axis=0, keepdims=True)
        tok = lax.broadcasted_iota(jnp.int32, (RC, 1), 0) + i * RC
        first = jnp.min(jnp.where(r == rmax, tok, S), axis=0, keepdims=True)
        if best is None:
            return rmax, first
        take = rmax > best[0]
        return jnp.where(take, rmax, best[0]), jnp.where(take, first, best[1])

    best, sent, out_cp = None, 0, []
    transpose_o(0)
    project(0)
    for i in range(NB):
        if i + 1 < NB:
            transpose_o(i + 1)
            project(i + 1)
        best = norm_and_score(i, best)
        if i in OUT_DMA_AFTER:
            rows = pl.ds(sent * RC, (i + 1 - sent) * RC)
            out_cp.append(pltpu.make_async_copy(out_v.at[rows, :], out_hbm.at[rows, :],
                                                osems.at[len(out_cp)]))
            out_cp[-1].start()
            sent = i + 1

    rmax, tok = best
    idx = jnp.minimum(jnp.max(tok), S - 1)
    t0 = pl.multiple_of((idx // 16) * 16, 16)
    ht = h_v[pl.ds(t0, 16), :]
    lnt = _ln(ht)
    sel = lax.broadcasted_iota(jnp.int32, (16, D), 0) == idx - t0
    xs = jnp.sum(jnp.where(sel, lnt, 0.0), axis=0, keepdims=True)
    xs = jnp.broadcast_to(xs, (16, D)).astype(bf16)
    g = jnp.dot(xs, wg_v[...], preferred_element_type=f32)
    u = jnp.dot(xs, wu_v[...], preferred_element_type=f32)
    act = (g * jax.nn.sigmoid(g) * u).astype(bf16)
    y = jnp.dot(act, wd_v[...], preferred_element_type=f32) * jax.nn.sigmoid(rmax)
    fix_v[...] = (ht + lnt + jnp.where(sel, y, 0.0)).astype(bf16)
    for c in out_cp:
        c.wait()
    fix_cp = pltpu.make_async_copy(fix_v, out_hbm.at[pl.ds(t0, 16), :], osems.at[len(out_cp)])
    fix_cp.start()
    fix_cp.wait()


@jax.jit
def pallas_sequential_preLN__mha_block__moe_arch_mod__prompt_kernel(
    A_x: jax.Array,
    A_wqkv: jax.Array,
    A_wo: jax.Array,
    B_x: jax.Array,
    B_w_r: jax.Array,
    B_w_gate: jax.Array,
    B_w_up: jax.Array,
    B_w_down: jax.Array,
):
    del B_x
    hbm = pl.BlockSpec(memory_space=pl.ANY)
    out = pl.pallas_call(
        _kernel,
        in_specs=[hbm] * 7,
        out_specs=hbm,
        out_shape=jax.ShapeDtypeStruct((S, D), bf16),
        scratch_shapes=[
            pltpu.VMEM((S, D), bf16),
            pltpu.VMEM((D, 3 * D), bf16),
            pltpu.VMEM((D, D), bf16),
            pltpu.VMEM((D,), bf16),
            pltpu.VMEM((D, F), bf16),
            pltpu.VMEM((D, F), bf16),
            pltpu.VMEM((F, D), bf16),
            pltpu.VMEM((D // 2, D), jnp.int32),
            pltpu.VMEM((S // 2, D), jnp.int32),
            pltpu.VMEM((2 * NW - 1, S // 2, 128), jnp.int32),
            pltpu.VMEM((2 * NW - 1, S // 2, 128), jnp.int32),
            pltpu.VMEM((D, S), f32),
            pltpu.VMEM((D, S), f32),
            pltpu.VMEM((S, D), f32),
            pltpu.VMEM((S, D), bf16),
            pltpu.VMEM((16, D), bf16),
            pltpu.VMEM((CK, CQ), f32),
            pltpu.VMEM((CK // 2, CQ), jnp.int32),
            pltpu.VMEM((40, CQ), f32),
            pltpu.VMEM((CQ // 2, 128), jnp.int32),
            pltpu.SemaphoreType.DMA((S // RA + 8,)),
            pltpu.SemaphoreType.DMA((len(OUT_DMA_AFTER) + 1,)),
        ],
        compiler_params=pltpu.CompilerParams(vmem_limit_bytes=100 * 1024 * 1024),
        name="preln_mha_mod_block",
    )(A_x.reshape(S, D), A_wqkv, A_wo, B_w_r, B_w_gate, B_w_up, B_w_down)
    return out.reshape(1, S, D)
```

```python
import math

import jax
import jax.numpy as jnp
from jax import lax
import jax.experimental.pallas as pl
import jax.experimental.pallas.tpu as pltpu

S, D, H, F = 2048, 640, 32, 1536
Dh = D // H
NW = D // 128
CQ, CK = 512, 128
NJ, NC = S // CQ, S // CK
HB = 2
RA, SB = 512, 256
RC = 128
OUT_DMA_AFTER = (7, 14, 15)
EPS = 1e-5
EPS_BF16 = 1.0013580322265625e-05
QSCALE = math.log2(math.e) * Dh ** -0.5
NT = (((1,), (1,)), ((), ()))
f32, bf16 = jnp.float32, jnp.bfloat16


def _ln(x):
    xc = x - jnp.mean(x, axis=-1, keepdims=True)
    return xc * lax.rsqrt(jnp.mean(xc * xc, axis=-1, keepdims=True) + EPS)


def _rb(x):
    return x.astype(bf16).astype(f32)


def _ln_bf16(x):
    mean = jnp.mean(x, axis=-1, keepdims=True)
    mean_b = _rb(mean)
    xc = x - mean_b
    var = jnp.mean(xc * xc, axis=-1, keepdims=True) - (mean - mean_b) * (mean - mean_b)
    sd = _rb(jnp.sqrt(_rb(_rb(var) + EPS_BF16)))
    return (_rb(xc) * pltpu.reciprocal(sd, approx=False)).astype(bf16)


def _pk(x):
    return pltpu.bitcast(x, jnp.int32)


def _unpk(x):
    return pltpu.bitcast(x, bf16)


def _store_shifted(dst, rows, wins):
    lane = lax.broadcasted_iota(jnp.int32, wins[0].shape, 1)
    rolled = [pltpu.roll(w, 64, 1) for w in wins]
    for w in range(NW - 1):
        dst[NW + w, rows, :] = jnp.where(lane < 64, rolled[w], rolled[w + 1])


def _store_windows(dst, r0, nr, val, shifted):
    rows = pl.ds(r0 // 2, nr // 2)
    wins = [_pk(val[:, 128 * w:128 * (w + 1)]) for w in range(NW)]
    for w in range(NW):
        dst[w, rows, :] = wins[w]
    if shifted:
        _store_shifted(dst, rows, wins)


def _attention(qw, kw, vt, ot, s_c, p_c, st_c, q_c, before_loop):
    items = [(j, c) for j in range(NJ) for c in range(NC)]
    NI = len(items)
    lane = lax.broadcasted_iota(jnp.int32, (CQ // 2, 128), 1)
    row8 = lax.broadcasted_iota(jnp.int32, (8, CK), 0)
    row24 = lax.broadcasted_iota(jnp.int32, (24, CQ), 0)
    st_m = st_c.at[pl.ds(0, 8), :]
    st_acc = st_c.at[pl.ds(8, 24), :]
    st_al = st_c.at[pl.ds(32, 8), :]

    class Head:
        def __init__(self, h, odd, valid=None):
            start = h * Dh
            w = start // 128
            off = start - w * 128
            straddles = off > 128 - Dh
            self.win = jnp.where(straddles, w + NW, w)
            self.off = jnp.where(straddles, off - 64, off)
            self.odd = odd
            self.vstart = pl.multiple_of((h // 2) * 40 + odd * 16, 8)
            self.valid = valid
            self.first = False
            self.qm, self.qj = None, -1
            self.m = self.acc = None

        def masked_q(self, j):
            q = qw[self.win, j * (CQ // 2):(j + 1) * (CQ // 2), :]
            mine = (lane >= self.off) & (lane < self.off + Dh)
            return jnp.where(mine, q, 0)

        def qk(self, n):
            j, c = items[n]
            if self.qj != j:
                self.qm, self.qj = _unpk(q_c[...] if (self.first and j == 0) else self.masked_q(j)), j
            k = _unpk(kw[self.win, c * (CK // 2):(c + 1) * (CK // 2), :])
            return lax.dot_general(k, self.qm, NT, preferred_element_type=f32)

        def softmax(self, n, s):
            _, c = items[n]
            cm = jnp.max(s, axis=0, keepdims=True)
            if c == 0:
                m, al = cm, None
            else:
                m = jnp.maximum(self.m, cm)
                al = jnp.exp2(self.m - m)
            self.m = m
            return jnp.exp2(s - m).astype(bf16), al

        def pv(self, n, p, al):
            j, c = items[n]
            v = vt[pl.ds(self.vstart, 24), c * CK:(c + 1) * CK]
            if self.odd:
                v = jnp.concatenate([jnp.where(row8 == 0, 1.0, v[:8]), v[8:]], axis=0)
            else:
                v = jnp.concatenate([v[:16], jnp.where(row8 == 4, 1.0, v[16:])], axis=0)
            r = jnp.dot(v, p, preferred_element_type=f32)
            self.acc = r if c == 0 else self.acc * al + r
            if c == NC - 1:
                l = self.acc[0:1, :] if self.odd else self.acc[20:21, :]
                o = self.acc * pltpu.reciprocal(l, approx=False)
                mine = row24 >= 4 if self.odd else row24 < Dh
                if self.valid is not None:
                    mine = mine & self.valid
                pltpu.store(ot.at[pl.ds(self.vstart, 24), j * CQ:(j + 1) * CQ], o, mask=mine)
                self.acc = None

    def load_state(prev):
        prev.m = st_m[0:1, :]
        prev.acc = st_acc[...]
        return s_c[...], (_unpk(p_c[...]), st_al[0:1, :])

    def body(i, carry):
        h0 = i * HB
        prev = Head(jnp.maximum(h0 - 1, 0), 1, valid=i > 0)
        heads = [Head(h0 + k, k % 2) for k in range(HB)]
        heads[0].first = True
        seq = [(prev, NI - 2), (prev, NI - 1)] + [(hd, n) for hd in heads for n in range(NI)]
        ss, pp = {}, {}
        ss[1], pp[0] = load_state(prev)
        for t in range(2, len(seq)):
            if t == 2:
                prev.pv(NI - 2, *pp.pop(0))
            hd, n = seq[t]
            ss[t] = hd.qk(n)
            hd, n = seq[t - 1]
            pp[t - 1] = hd.softmax(n, ss.pop(t - 1))
            if t > 2:
                hd, n = seq[t - 2]
                hd.pv(n, *pp.pop(t - 2))
        last = heads[-1]
        s_c[...] = ss.pop(len(seq) - 1)
        p, al = pp.pop(len(seq) - 2)
        p_c[...] = _pk(p)
        st_al[...] = jnp.broadcast_to(al, (8, CQ))
        st_m[...] = jnp.broadcast_to(last.m, (8, CQ))
        st_acc[...] = last.acc
        q_c[...] = Head(jnp.minimum(h0 + HB, H - 1), 0).masked_q(0)
        return carry

    q_c[...] = Head(0, 0).masked_q(0)
    before_loop()
    lax.fori_loop(0, H // HB, body, 0)
    last = Head(H - 1, 1)
    s, (p, al) = load_state(last)
    tail = last.softmax(NI - 1, s)
    last.pv(NI - 2, p, al)
    last.pv(NI - 1, *tail)


def _kernel(x_hbm, wqkv_hbm, wo_hbm, wr_hbm, wg_hbm, wu_hbm, wd_hbm, out_hbm,
            x_v, wqkv_v, wo_v, wr_v, wg_v, wu_v, wd_v,
            wvt_v, a_v, qw, kw, vt, ot, h_v, out_v, fix_v, s_c, p_c, st_c, q_c, sems, osems):
    NA, NB = S // RA, S // RC
    cp_x = [pltpu.make_async_copy(x_hbm.at[pl.ds(i * RA, RA), :], x_v.at[pl.ds(i * RA, RA), :],
                                  sems.at[i]) for i in range(NA)]
    cp_w = [pltpu.make_async_copy(wqkv_hbm.at[:, pl.ds(i * D, D)], wqkv_v.at[:, pl.ds(i * D, D)],
                                  sems.at[NA + i]) for i in range(3)]
    rest = [pltpu.make_async_copy(src, dst, sems.at[NA + 3 + i]) for i, (src, dst) in enumerate(
        [(wo_hbm, wo_v), (wr_hbm, wr_v), (wg_hbm, wg_v), (wu_hbm, wu_v), (wd_hbm, wd_v)])]
    for c in (cp_x[0], cp_w[0], cp_w[1], cp_x[1], cp_w[2], cp_x[2], cp_x[3]):
        c.start()

    def lhs(r0, nr):
        return _unpk(a_v[r0 // 2:(r0 + nr) // 2, :])

    def do_ln(i):
        a_v[i * (RA // 2):(i + 1) * (RA // 2), :] = _pk(_ln_bf16(x_v[i * RA:(i + 1) * RA, :].astype(f32)))

    def do_q(i, shifted=True):
        for r0 in range(i * RA, (i + 1) * RA, SB):
            q = jnp.dot(lhs(r0, SB), wqkv_v[:, 0:D], preferred_element_type=f32) * QSCALE
            _store_windows(qw, r0, SB, q.astype(bf16), shifted)

    def shift_q(i):
        rows = pl.ds(i * (RA // 2), RA // 2)
        _store_shifted(qw, rows, [qw[w, rows, :] for w in range(NW)])

    def do_k(i):
        for r0 in range(i * RA, (i + 1) * RA, SB):
            k = jnp.dot(lhs(r0, SB), wqkv_v[:, D:2 * D], preferred_element_type=f32)
            _store_windows(kw, r0, SB, k.astype(bf16), True)

    def do_v(i):
        for r0 in range(i * RA, (i + 1) * RA, SB):
            vt[:, r0:r0 + SB] = lax.dot_general(_unpk(wvt_v[...]), lhs(r0, SB), NT,
                                                preferred_element_type=f32)

    s_c[...] = jnp.zeros(s_c.shape, f32)
    p_c[...] = jnp.zeros(p_c.shape, jnp.int32)
    st_c[...] = jnp.ones(st_c.shape, f32)
    cp_x[0].wait()
    do_ln(0)
    cp_w[0].wait()
    do_q(0, False)
    cp_w[1].wait()
    cp_x[1].wait()
    do_ln(1)
    do_k(0)
    shift_q(0)
    do_q(1, False)
    cp_w[2].wait()
    cp_x[2].wait()
    cp_x[3].wait()
    for c in rest:
        c.start()
    wvt_v[...] = _pk(wqkv_v[:, 2 * D:3 * D].T)
    do_k(1)
    do_ln(2)
    shift_q(1)
    do_v(0)
    do_v(1)
    for i in range(2, NA):
        do_q(i)
        if i + 1 < NA:
            do_ln(i + 1)
        do_k(i)
        do_v(i)

    def wait_rest():
        for c in rest:
            c.wait()

    _attention(qw, kw, vt, ot, s_c, p_c, st_c, q_c, wait_rest)

    wr = wr_v[...].astype(f32).reshape(1, D)

    def transpose_o(i):
        a_v[i * (RC // 2):(i + 1) * (RC // 2), :] = _pk(ot[:, i * RC:(i + 1) * RC].astype(bf16).T)

    def project(i):
        rows = pl.ds(i * RC, RC)
        h_v[rows, :] = x_v[rows, :].astype(f32) + jnp.dot(
            lhs(i * RC, RC), wo_v[...], preferred_element_type=f32)

    def norm_and_score(i, best):
        rows = pl.ds(i * RC, RC)
        h = h_v[rows, :]
        lnh = _ln(h)
        out_v[rows, :] = (h + lnh).astype(bf16)
        r = jnp.sum(lnh.astype(bf16).astype(f32) * wr, axis=-1, keepdims=True)
        rmax = jnp.max(r, axis=0, keepdims=True)
        tok = lax.broadcasted_iota(jnp.int32, (RC, 1), 0) + i * RC
        first = jnp.min(jnp.where(r == rmax, tok, S), axis=0, keepdims=True)
        if best is None:
            return rmax, first
        take = rmax > best[0]
        return jnp.where(take, rmax, best[0]), jnp.where(take, first, best[1])

    best, sent, out_cp = None, 0, []
    transpose_o(0)
    project(0)
    for i in range(NB):
        if i + 1 < NB:
            transpose_o(i + 1)
            project(i + 1)
        best = norm_and_score(i, best)
        if i in OUT_DMA_AFTER:
            rows = pl.ds(sent * RC, (i + 1 - sent) * RC)
            out_cp.append(pltpu.make_async_copy(out_v.at[rows, :], out_hbm.at[rows, :],
                                                osems.at[len(out_cp)]))
            out_cp[-1].start()
            sent = i + 1

    rmax, tok = best
    idx = jnp.minimum(jnp.max(tok), S - 1)
    t0 = pl.multiple_of((idx // 16) * 16, 16)
    ht = h_v[pl.ds(t0, 16), :]
    lnt = _ln(ht)
    sel = lax.broadcasted_iota(jnp.int32, (16, D), 0) == idx - t0
    xs = jnp.sum(jnp.where(sel, lnt, 0.0), axis=0, keepdims=True)
    xs = jnp.broadcast_to(xs, (16, D)).astype(bf16)
    g = jnp.dot(xs, wg_v[...], preferred_element_type=f32)
    u = jnp.dot(xs, wu_v[...], preferred_element_type=f32)
    act = (g * jax.nn.sigmoid(g) * u).astype(bf16)
    y = jnp.dot(act, wd_v[...], preferred_element_type=f32) * jax.nn.sigmoid(rmax)
    fix_v[...] = (ht + lnt + jnp.where(sel, y, 0.0)).astype(bf16)
    for c in out_cp:
        c.wait()
    fix_cp = pltpu.make_async_copy(fix_v, out_hbm.at[pl.ds(t0, 16), :], osems.at[len(out_cp)])
    fix_cp.start()
    fix_cp.wait()


@jax.jit
def pallas_sequential_preLN__mha_block__moe_arch_mod__prompt_kernel(
    A_x: jax.Array,
    A_wqkv: jax.Array,
    A_wo: jax.Array,
    B_x: jax.Array,
    B_w_r: jax.Array,
    B_w_gate: jax.Array,
    B_w_up: jax.Array,
    B_w_down: jax.Array,
):
    del B_x
    hbm = pl.BlockSpec(memory_space=pl.ANY)
    out = pl.pallas_call(
        _kernel,
        in_specs=[hbm] * 7,
        out_specs=hbm,
        out_shape=jax.ShapeDtypeStruct((S, D), bf16),
        scratch_shapes=[
            pltpu.VMEM((S, D), bf16),
            pltpu.VMEM((D, 3 * D), bf16),
            pltpu.VMEM((D, D), bf16),
            pltpu.VMEM((D,), bf16),
            pltpu.VMEM((D, F), bf16),
            pltpu.VMEM((D, F), bf16),
            pltpu.VMEM((F, D), bf16),
            pltpu.VMEM((D // 2, D), jnp.int32),
            pltpu.VMEM((S // 2, D), jnp.int32),
            pltpu.VMEM((2 * NW - 1, S // 2, 128), jnp.int32),
            pltpu.VMEM((2 * NW - 1, S // 2, 128), jnp.int32),
            pltpu.VMEM((D, S), f32),
            pltpu.VMEM((D, S), f32),
            pltpu.VMEM((S, D), f32),
            pltpu.VMEM((S, D), bf16),
            pltpu.VMEM((16, D), bf16),
            pltpu.VMEM((CK, CQ), f32),
            pltpu.VMEM((CK // 2, CQ), jnp.int32),
            pltpu.VMEM((40, CQ), f32),
            pltpu.VMEM((CQ // 2, 128), jnp.int32),
            pltpu.SemaphoreType.DMA((S // RA + 8,)),
            pltpu.SemaphoreType.DMA((len(OUT_DMA_AFTER) + 1,)),
        ],
        compiler_params=pltpu.CompilerParams(vmem_limit_bytes=100 * 1024 * 1024),
        name="preln_mha_mod_block",
    )(A_x.reshape(S, D), A_wqkv, A_wo, B_w_r, B_w_gate, B_w_up, B_w_down)
    return out.reshape(1, S, D)
```
